```python
import os as _os
_os.environ.setdefault("JAX_PLATFORMS", "cpu")
import jax
import jax.numpy as jnp

def _softmax(x, axis=-1):
    return jax.nn.softmax(x, axis=axis)
def _gelu(x):
    return jax.nn.gelu(x, approximate=True)
def _silu(x):
    return jax.nn.silu(x)
def _sigmoid(x):
    return jax.nn.sigmoid(x)
def _layernorm(x, axis=-1, eps=1e-5):
    m = jnp.mean(x, axis=axis, keepdims=True)
    v = jnp.var(x, axis=axis, keepdims=True)
    return (x - m) / jnp.sqrt(v + eps)
def _scatter_add(tgt, idx, src, axis=0):
    return tgt.at[idx].add(src)
def _segment_sum(src, seg, n):
    return jax.ops.segment_sum(src, seg, n)
class _Rng:
    def __init__(self, key):
        self._k = key
    def _next(self):
        self._k, sub = jax.random.split(self._k)
        return sub
    def normal(self, shape):
        return jax.random.normal(self._next(), shape, dtype=jnp.bfloat16)
    def randint(self, lo, hi, shape):
        return jax.random.randint(self._next(), shape, lo, hi, dtype=jnp.int32)
    def uniform(self, shape, lo=0.0, hi=1.0):
        return jax.random.uniform(self._next(), shape, jnp.bfloat16, lo, hi)
    def permutation(self, n):
        return jax.random.permutation(self._next(), n)


kernel_name = 'sequential_preLN__mha_block__swiglu_ffn__prompt'

def setup_inputs():
    _rng = _Rng(jax.random.key(int.from_bytes(__import__("os").urandom(4), "little")))
    _w = (lambda a: (lambda t: t.astype(jnp.bfloat16) if jnp.issubdtype(t.dtype, jnp.floating) else t)(jnp.asarray(a)))
    def _A_setup():
        B, S, D, H = 1, 2048, 640, 32
        return {
            "x": _w((lambda *s: _rng.normal(s) * 0.05)(B, S, D)),
            "wqkv": _w((lambda *s: _rng.normal(s) * 0.05)(D, 3 * D)),
            "wo": _w((lambda *s: _rng.normal(s) * 0.05)(D, D)),
        }
    _A_in = _A_setup()

    def _B_setup():
        B, S, D, F = 1, 2048, 640, 1728
        return {
            "x": _w((lambda *s: _rng.normal(s) * 0.05)(B, S, D)),
            "w_gate": _w((lambda *s: _rng.normal(s) * 0.05)(D, F)),
            "w_up": _w((lambda *s: _rng.normal(s) * 0.05)(D, F)),
            "w_down": _w((lambda *s: _rng.normal(s) * 0.05)(F, D)),
        }
    _B_in = _B_setup()

    return {
        "A_x": _A_in["x"],
        "A_wqkv": _A_in["wqkv"],
        "A_wo": _A_in["wo"],
        "B_x": _B_in["x"],
        "B_w_gate": _B_in["w_gate"],
        "B_w_up": _B_in["w_up"],
        "B_w_down": _B_in["w_down"],
    }

def reference(A_x, A_wqkv, A_wo, B_x, B_w_gate, B_w_up, B_w_down):
    def _A_ref(x, wqkv, wo):
        B, S, D = x.shape
        H = 32
        Dh = D // H
        qkv = (lambda x, *d: x.transpose(*d))((x @ wqkv).reshape(B, S, 3, H, Dh), 2, 0, 3, 1, 4)
        q, k, v = qkv[0], qkv[1], qkv[2]
        scores = jnp.einsum("bhqd,bhkd->bhqk", q, k) * (Dh ** -0.5)
        p = _softmax(scores, axis=-1)
        o = jnp.einsum("bhqk,bhkd->bhqd", p, v)
        return (lambda x, *d: x.transpose(*d))(o, 0, 2, 1, 3).reshape(B, S, D) @ wo

    def _B_ref(x, w_gate, w_up, w_down):
        g = _silu(x @ w_gate)
        u = x @ w_up
        return (g * u) @ w_down

    x = A_x
    h = x + _A_ref(_layernorm(x, axis=-1), A_wqkv, A_wo)
    h2 = h + _B_ref(_layernorm(h, axis=-1), B_w_gate, B_w_up, B_w_down)
    return h2
```

```python
import functools
import jax, jax.numpy as jnp, numpy as np
from jax import lax
from jax.experimental import pallas as pl
from jax.experimental.pallas import tpu as pltpu

S, D, H, DH, F = 2048, 640, 32, 20, 1728
EPS = 1e-5
QSCALE = float(DH ** -0.5 * np.log2(np.e))
bf16, f32 = jnp.bfloat16, jnp.float32

def _ln(x):
    m = jnp.mean(x, axis=-1, keepdims=True)
    c = x - m
    v = jnp.mean(c * c, axis=-1, keepdims=True)
    return c * lax.rsqrt(v + EPS)

def make(TQ=512, PIPE=True, UNROLL=1, RC=512, flags=None):
    NQ = S // TQ
    def kernel(x_ref, wqkv_ref, wo_ref, wg_ref, wu_ref, wd_ref, o_ref,
               q_scr, k_scr, vt_scr, s_scr, at_scr):
        i = pl.program_id(0)

        @pl.when(i == 0)
        def _phase1():
            def chunk(c, _):
                r0 = pl.multiple_of(c * RC, RC)
                xn = _ln(x_ref[pl.ds(r0, RC), :].astype(f32)).astype(bf16)
                q = jnp.dot(xn, wqkv_ref[:, 0:D], preferred_element_type=f32) * QSCALE
                for a in range(5):
                    q_scr[a, pl.ds(r0, RC), :] = q[:, a*128:(a+1)*128].astype(bf16)
                k = jnp.dot(xn, wqkv_ref[:, D:2*D], preferred_element_type=f32)
                lane = lax.broadcasted_iota(jnp.int32, (RC, 128), 1)
                for a in range(5):
                    ka = k[:, a*128:(a+1)*128]
                    k_scr[2*a, pl.ds(r0, RC), :] = ka.astype(bf16)
                    if a < 4:
                        kb = k[:, (a+1)*128:(a+2)*128]
                        k_scr[2*a+1, pl.ds(r0, RC), :] = jnp.where(lane >= 64, ka, kb).astype(bf16)
                v = jnp.dot(xn, wqkv_ref[:, 2*D:3*D], preferred_element_type=f32)
                vt = v.T
                ones = jnp.ones((8, RC), f32)
                for h in range(H):
                    st = (h * DH) // 8 * 8
                    vt_scr[h, :, pl.ds(r0, RC)] = jnp.concatenate([vt[st:st+24], ones], axis=0).astype(bf16)
                return 0
            lax.fori_loop(0, S // RC, chunk, 0)

        q0 = pl.multiple_of(i * TQ, TQ)
        lane = lax.broadcasted_iota(jnp.int32, (TQ, 128), 1)

        def qk(h, slot):
            lo = h * DH
            a = lo // 128
            b = (lo + DH - 1) // 128
            l0 = lo % 128
            qa = q_scr[a, pl.ds(q0, TQ), :]
            qb = q_scr[b, pl.ds(q0, TQ), :]
            rel = (lane - l0) & 127
            qm = jnp.where(rel < DH, jnp.where(lane >= l0, qa, qb), jnp.zeros_like(qa))
            s = lax.dot_general(k_scr[a + b], qm, (((1,), (1,)), ((), ())), preferred_element_type=f32)
            s_scr[slot] = s
            return jnp.max(s, axis=0, keepdims=True)

        def pv(h, slot, m):
            p = jnp.exp2(s_scr[slot] - m).astype(bf16)
            o = jnp.dot(vt_scr[h], p, preferred_element_type=f32)
            return o[0:24] * (1.0 / o[24:25])

        row = lax.broadcasted_iota(jnp.int32, (8, TQ), 0)
        def store_pair(j, oe, oo):
            r = pl.multiple_of(j * 40, 8)
            at_scr[pl.ds(r, 16), :] = oe[0:16]
            at_scr[pl.ds(r + 16, 8), :] = jnp.where(row < 4, oe[16:24], oo[0:8])
            at_scr[pl.ds(r + 24, 16), :] = oo[8:24]

        if PIPE:
            m0 = qk(0, 0)
            def body(j, m0):
                m1 = qk(2*j + 1, 1)
                oe = pv(2*j, 0, m0)
                m2 = qk(jnp.minimum(2*j + 2, H - 1), 0)
                oo = pv(2*j + 1, 1, m1)
                store_pair(j, oe, oo)
                return m2
            lax.fori_loop(0, H // 2, body, m0, unroll=UNROLL)
        else:
            def body(j, c):
                m0 = qk(2*j, 0)
                m1 = qk(2*j + 1, 1)
                oe = pv(2*j, 0, m0)
                oo = pv(2*j + 1, 1, m1)
                store_pair(j, oe, oo)
                return c
            lax.fori_loop(0, H // 2, body, 0, unroll=UNROLL)

        at = at_scr[...].astype(bf16)
        hres = x_ref[pl.ds(q0, TQ), :].astype(f32) + lax.dot_general(
            at, wo_ref[...], (((0,), (0,)), ((), ())), preferred_element_type=f32)
        hn = _ln(hres).astype(bf16)
        g = jnp.dot(hn, wg_ref[...], preferred_element_type=f32)
        u = jnp.dot(hn, wu_ref[...], preferred_element_type=f32)
        act = (g * jax.nn.sigmoid(g) * u).astype(bf16)
        o_ref[...] = (hres + jnp.dot(act, wd_ref[...], preferred_element_type=f32)).astype(o_ref.dtype)

    full = lambda shape: pl.BlockSpec(shape, lambda i: (0,) * len(shape), pipeline_mode=pl.Buffered(1))
    def fn(A_x, A_wqkv, A_wo, B_x, B_w_gate, B_w_up, B_w_down):
        out = pl.pallas_call(
            kernel,
            grid=(NQ,),
            in_specs=[full((S, D)), full((D, 3*D)), full((D, D)), full((D, F)), full((D, F)), full((F, D))],
            out_specs=pl.BlockSpec((TQ, D), lambda i: (i, 0)),
            out_shape=jax.ShapeDtypeStruct((S, D), A_x.dtype),
            scratch_shapes=[pltpu.VMEM((5, S, 128), bf16), pltpu.VMEM((9, S, 128), bf16),
                            pltpu.VMEM((H, 32, S), bf16), pltpu.VMEM((2, S, TQ), f32),
                            pltpu.VMEM((D, TQ), f32)],
            compiler_params=pltpu.CompilerParams(dimension_semantics=("arbitrary",),
                                                 vmem_limit_bytes=110 * 2**20, flags=flags),
        )(A_x.reshape(S, D), A_wqkv, A_wo, B_w_gate, B_w_up, B_w_down)
        return out.reshape(1, S, D)
    return fn


_impl = make(512, True)


@jax.jit
def pallas_sequential_preLN__mha_block__swiglu_ffn__prompt_kernel(
    A_x, A_wqkv, A_wo, B_x, B_w_gate, B_w_up, B_w_down
):
    return _impl(A_x, A_wqkv, A_wo, B_x, B_w_gate, B_w_up, B_w_down)
```

```python
import jax, jax.numpy as jnp, numpy as np
from jax import lax
from jax.experimental import pallas as pl
from jax.experimental.pallas import tpu as pltpu

S, D, H, DH, F = 2048, 640, 32, 20, 1728
EPS = 1e-5
QSCALE = float(DH ** -0.5 * np.log2(np.e))
bf16, f32 = jnp.bfloat16, jnp.float32
NN = (((1,), (0,)), ((), ()))
NT = (((1,), (1,)), ((), ()))
TN = (((0,), (0,)), ((), ()))
TQ, KC = 512, 128
NQ = S // TQ

def _dot(a, b, dims=NN):
    return lax.dot_general(a, b, dims, preferred_element_type=f32)

def _ln(x):
    m = jnp.mean(x, axis=-1, keepdims=True)
    c = x - m
    v = jnp.mean(c * c, axis=-1, keepdims=True)
    return c * lax.rsqrt(v + EPS)

def make(UN=7, RC=512, TF=512, TS=2, QT=True, P1=1, CAT=True, PF=True, flags=None):
    NC = S // RC
    NF = S // TF
    def kernel(x_hbm, wqkv_hbm, wo_hbm, wg_hbm, wu_hbm, wd_hbm, o_hbm,
               x_ref, wqkv_ref, wo_ref, wg_ref, wu_ref, wd_ref,
               q_scr, k_scr, vt_scr, s_scr, at_scr, h_scr, hn_scr, o_scr, xsem, wsem, osem):
        xcp = [pltpu.make_async_copy(x_hbm.at[pl.ds(c * RC, RC)], x_ref.at[pl.ds(c * RC, RC)], xsem.at[c])
               for c in range(NC)]
        wcp = [pltpu.make_async_copy(wqkv_hbm.at[:, pl.ds(n * D, D)], wqkv_ref.at[:, pl.ds(n * D, D)], wsem.at[n]) for n in range(3)]
        fcp = [pltpu.make_async_copy(a, b, wsem.at[3 + n]) for n, (a, b) in enumerate(
            ((wo_hbm, wo_ref), (wg_hbm, wg_ref), (wu_hbm, wu_ref), (wd_hbm, wd_ref)))]

        xcp[0].start()
        wcp[0].start()
        xcp[0].wait()
        wcp[1].start()
        lane = lax.broadcasted_iota(jnp.int32, (RC, 128), 1)
        row = lax.broadcasted_iota(jnp.int32, (8, RC), 0)
        def chunk(c, _):
            first = isinstance(c, int)
            rs = pl.ds(c * RC if first else pl.multiple_of(c * RC, RC), RC)
            def once(f):
                if first: f()
                elif P1 == 0: pl.when(c == 0)(f)
            if first:
                xn = _ln(x_ref[rs, :].astype(f32)).astype(bf16)
            else:
                xn = hn_scr[rs, :]
            @once
            def _():
                wcp[0].wait()
                wcp[2].start()
            if first or not CAT:
                proj = lambda n: _dot(xn, wqkv_ref[:, n * D:(n + 1) * D])
            else:
                qkv = _dot(xn, wqkv_ref[...])
                proj = lambda n: qkv[:, n * D:(n + 1) * D]
            q = proj(0) * QSCALE
            if QT:
                qt = q.T
                for a in range(5):
                    q_scr[a, :, rs] = qt[a*128:(a+1)*128].astype(bf16)
            else:
                for a in range(5):
                    q_scr[a, rs, :] = q[:, a*128:(a+1)*128].astype(bf16)
            @once
            def _():
                wcp[1].wait()
                xcp[1].start()
            k = proj(1)
            for a in range(5):
                ka = k[:, a*128:(a+1)*128]
                k_scr[2*a, rs, :] = ka.astype(bf16)
                if a < 4:
                    kb = k[:, (a+1)*128:(a+2)*128]
                    k_scr[2*a+1, rs, :] = jnp.where(lane >= 64, ka, kb).astype(bf16)
            @once
            def _():
                wcp[2].wait()
                xcp[1].wait()
                for cp in xcp[2:]:
                    cp.start()
            n0 = RC if first else pl.multiple_of(jnp.where(c + 1 < NC, c + 1, 0) * RC, RC)
            hn_scr[pl.ds(n0, RC), :] = _ln(x_ref[pl.ds(n0, RC), :].astype(f32)).astype(bf16)
            vt = proj(2).T
            for h in range(H):
                st = (h * DH) // 8 * 8
                if h % 2 == 0:
                    vt_scr[h, 0:16, rs] = vt[st:st+16]
                    vt_scr[h, 16:24, rs] = jnp.where(row < 4, vt[st+16:st+24], 1.0)
                else:
                    vt_scr[h, 0:8, rs] = jnp.where(row < 4, 1.0, vt[st:st+8])
                    vt_scr[h, 8:24, rs] = vt[st+8:st+24]
            @once
            def _():
                for cp in xcp[2:]:
                    cp.wait()
                for cp in fcp:
                    cp.start()
            return 0
        if P1 == 1:
            chunk(0, 0)
        lax.fori_loop(P1, NC, chunk, 0)

        if QT:
            lane = lax.broadcasted_iota(jnp.int32, (128, TQ), 0)
        else:
            lane = lax.broadcasted_iota(jnp.int32, (TQ, 128), 1)

        def tile_start(n):
            return (n // H) * TQ if isinstance(n, int) else pl.multiple_of((n // H) * TQ, TQ)

        def getq(n):
            q0 = tile_start(n)
            lo = (n % H) * DH
            a = lo // 128
            b = (lo + DH - 1) // 128
            l0 = lo % 128
            if QT:
                qa = q_scr[a, :, pl.ds(q0, TQ)]
                qb = q_scr[b, :, pl.ds(q0, TQ)]
            else:
                qa = q_scr[a, pl.ds(q0, TQ), :]
                qb = q_scr[b, pl.ds(q0, TQ), :]
            rel = (lane - l0) & 127
            qm = jnp.where(rel < DH, jnp.where(lane >= l0, qa, qb), jnp.zeros_like(qa))
            return qm, a + b

        def step(nn, sn, n, sc, m):
            mx = o = None
            if nn is not None:
                qm, ki = getq(nn)
            for c in range(S // KC):
                ks = slice(c * KC, (c + 1) * KC)
                if nn is not None:
                    s = _dot(k_scr[ki, ks, :], qm, NN if QT else NT)
                    s_scr[sn, ks, :] = s
                    sm = jnp.max(s.reshape(KC // 8, 8, TQ), axis=0)
                    mx = sm if mx is None else jnp.maximum(mx, sm)
                if n is not None:
                    p = jnp.exp2(s_scr[sc, ks, :] - m).astype(bf16)
                    d = _dot(vt_scr[n % H, :, ks], p)
                    o = d if o is None else o + d
            if mx is not None:
                mx = jnp.max(mx, axis=0, keepdims=True)
            if o is not None:
                lr = 20 if sc == 0 else 0
                o = o * (1.0 / o[lr:lr+1])
            return mx, o

        row = lax.broadcasted_iota(jnp.int32, (8, TQ), 0)
        def store_pair(j, oe, oo):
            r = (j % (H // 2)) * 40
            if not isinstance(j, int):
                r = pl.multiple_of(r, 8)
            cs = pl.ds(tile_start(2 * j), TQ)
            at_scr[pl.ds(r, 16), cs] = oe[0:16]
            at_scr[pl.ds(r + 16, 8), cs] = jnp.where(row < 4, oe[16:24], oo[0:8])
            at_scr[pl.ds(r + 24, 16), cs] = oo[8:24]

        m0, _ = step(0, 0, None, None, None)
        def body(j, m0):
            m1, oe = step(2*j + 1, 1, 2*j, 0, m0)
            m2, oo = step(2*j + 2, 0, 2*j + 1, 1, m1)
            store_pair(j, oe, oo)
            return m2
        NP = NQ * H // 2
        m0 = lax.fori_loop(0, NP - 1, body, m0, unroll=UN)
        for cp in fcp:
            cp.wait()

        def head(t0):
            T = TF // TS
            for t in range(TS):
                rs = pl.ds(t0 + t * T, T)
                h = x_ref[rs, :].astype(f32) + _dot(at_scr[:, rs].T.astype(bf16), wo_ref[...])
                h_scr[rs, :] = h
                hn_scr[rs, :] = _ln(h).astype(bf16)

        def ocp(i, t0):
            return pltpu.make_async_copy(o_scr.at[pl.ds(t0, TF)], o_hbm.at[pl.ds(t0, TF)], osem.at[i])

        def ffn(i, t0, nxt):
            rs = pl.ds(t0, TF)
            hn = hn_scr[rs, :]
            g = _dot(wg_ref[...], hn, NT)
            u = _dot(wu_ref[...], hn, NT)
            act = (g * jax.nn.sigmoid(g) * u).astype(bf16)
            if nxt:
                head(t0 + TF)
            o_scr[rs, :] = (h_scr[rs, :] + _dot(act, wd_ref[...], TN)).astype(o_scr.dtype)
            ocp(i, t0).start()

        m1, oe = step(2 * NP - 1, 1, 2 * NP - 2, 0, m0)
        if PF: head(0)
        _, oo = step(None, None, 2 * NP - 1, 1, m1)
        store_pair(NP - 1, oe, oo)
        def fbody(i, c):
            t0 = pl.multiple_of(i * TF, TF)
            if not PF: head(t0)
            ffn(i, t0, PF)
            return c
        lax.fori_loop(0, NF - 1 if PF else NF, fbody, 0)
        if PF: ffn(NF - 1, S - TF, False)
        for i in range(NF):
            ocp(i, i * TF).wait()

    hbm = pl.BlockSpec(memory_space=pltpu.HBM)
    def fn(A_x, A_wqkv, A_wo, B_x, B_w_gate, B_w_up, B_w_down):
        out = pl.pallas_call(
            kernel,
            in_specs=[hbm] * 6,
            out_specs=hbm,
            out_shape=jax.ShapeDtypeStruct((S, D), A_x.dtype),
            scratch_shapes=[pltpu.VMEM((S, D), bf16), pltpu.VMEM((D, 3 * D), bf16), pltpu.VMEM((D, D), bf16),
                            pltpu.VMEM((F, D), bf16), pltpu.VMEM((F, D), bf16), pltpu.VMEM((F, D), bf16),
                            pltpu.VMEM((5, 128, S) if QT else (5, S, 128), bf16), pltpu.VMEM((9, S, 128), bf16),
                            pltpu.VMEM((H, 24, S), f32), pltpu.VMEM((2, S, TQ), f32),
                            pltpu.VMEM((D, S), f32), pltpu.VMEM((S, D), f32), pltpu.VMEM((S, D), bf16),
                            pltpu.VMEM((S, D), bf16),
                            pltpu.SemaphoreType.DMA((NC,)), pltpu.SemaphoreType.DMA((7,)), pltpu.SemaphoreType.DMA((NF,))],
            compiler_params=pltpu.CompilerParams(vmem_limit_bytes=110 * 2**20, flags=flags),
        )(A_x.reshape(S, D), A_wqkv, A_wo, B_w_gate.T, B_w_up.T, B_w_down)
        return out.reshape(1, S, D)
    return fn


_impl = make(4, TF=256, TS=1)


@jax.jit
def pallas_sequential_preLN__mha_block__swiglu_ffn__prompt_kernel(
    A_x, A_wqkv, A_wo, B_x, B_w_gate, B_w_up, B_w_down
):
    return _impl(A_x, A_wqkv, A_wo, B_x, B_w_gate, B_w_up, B_w_down)
```
